```python
import os as _os
_os.environ.setdefault("JAX_PLATFORMS", "cpu")
import jax
import jax.numpy as jnp

def _softmax(x, axis=-1):
    return jax.nn.softmax(x, axis=axis)
def _gelu(x):
    return jax.nn.gelu(x, approximate=True)
def _silu(x):
    return jax.nn.silu(x)
def _sigmoid(x):
    return jax.nn.sigmoid(x)
def _layernorm(x, axis=-1, eps=1e-5):
    m = jnp.mean(x, axis=axis, keepdims=True)
    v = jnp.var(x, axis=axis, keepdims=True)
    return (x - m) / jnp.sqrt(v + eps)
def _scatter_add(tgt, idx, src, axis=0):
    return tgt.at[idx].add(src)
def _segment_sum(src, seg, n):
    return jax.ops.segment_sum(src, seg, n)
class _Rng:
    def __init__(self, key):
        self._k = key
    def _next(self):
        self._k, sub = jax.random.split(self._k)
        return sub
    def normal(self, shape):
        return jax.random.normal(self._next(), shape, dtype=jnp.bfloat16)
    def randint(self, lo, hi, shape):
        return jax.random.randint(self._next(), shape, lo, hi, dtype=jnp.int32)
    def uniform(self, shape, lo=0.0, hi=1.0):
        return jax.random.uniform(self._next(), shape, jnp.bfloat16, lo, hi)
    def permutation(self, n):
        return jax.random.permutation(self._next(), n)


kernel_name = 'gated_mix__sliding_block__dense_activation_silu__prompt'

def setup_inputs():
    _rng = _Rng(jax.random.key(int.from_bytes(__import__("os").urandom(4), "little")))
    _w = (lambda a: (lambda t: t.astype(jnp.bfloat16) if jnp.issubdtype(t.dtype, jnp.floating) else t)(jnp.asarray(a)))
    def _A_setup():
        B, S, D = 1, 2048, 640
        return {
            "x": _w((lambda *s: _rng.normal(s) * 0.05)(B, S, D)),
            "wqkv": _w((lambda *s: _rng.normal(s) * 0.4)(D, 3 * D)),
            "wo": _w((lambda *s: _rng.normal(s) * 0.05)(D, D)),
        }
    _A_in = _A_setup()

    def _B_setup():
        B, S, D, F = 1, 2048, 640, 1536
        return {
            "x": _w((lambda *s: _rng.normal(s) * 0.05)(B, S, D)),
            "w1": _w((lambda *s: _rng.normal(s) * 1.6)(D, F) * (D ** -0.5)),
            "w2": _w((lambda *s: _rng.normal(s) * 1.6)(F, D) * (F ** -0.5)),
        }
    _B_in = _B_setup()

    return {
        "A_x": _A_in["x"],
        "A_wqkv": _A_in["wqkv"],
        "A_wo": _A_in["wo"],
        "B_x": _B_in["x"],
        "B_w1": _B_in["w1"],
        "B_w2": _B_in["w2"],
        "gate_w": _w((lambda *s: _rng.normal(s) * 0.05)(640) * 16.0),
    }

def reference(A_x, A_wqkv, A_wo, B_x, B_w1, B_w2, gate_w):
    def _A_ref(x, wqkv, wo):
        B, S, D = x.shape
        H = 32; Dh = D // H; W = 256
        qkv = (lambda x, *d: x.transpose(*d))((x @ wqkv).reshape(B, S, 3, H, Dh), 2, 0, 3, 1, 4)
        q, k, v = qkv[0], qkv[1], qkv[2]
        scores = jnp.einsum("bhqd,bhkd->bhqk", q, k) * (Dh ** -0.5)
        idx = jnp.arange(S)
        mask = (idx[:, None] - idx[None, :] >= 0) & (idx[:, None] - idx[None, :] < W)
        scores = jnp.where(mask[None, None], scores, -1e9)
        p = _softmax(scores, axis=-1)
        o = jnp.einsum("bhqk,bhkd->bhqd", p, v)
        return (lambda x, *d: x.transpose(*d))(o, 0, 2, 1, 3).reshape(B, S, D) @ wo

    def _B_ref(x, w1, w2):
        h = jnp.einsum("bsd,df->bsf", x, w1)
        h = _silu(h)
        out = jnp.einsum("bsf,fd->bsd", h, w2)
        return out

    x = A_x
    g = _sigmoid((x * gate_w).sum(-1, keepdims=True))
    a = _A_ref(x, A_wqkv, A_wo)
    b = _B_ref(x, B_w1, B_w2)
    return g * a + (1 - g) * b
```

```python
import math

import jax
import jax.numpy as jnp
from jax import lax
import jax.experimental.pallas as pl
import jax.experimental.pallas.tpu as pltpu

S, D, F, H, DH, W = 2048, 640, 1536, 32, 20, 256
TQ = 512
SB = 128
NSB = TQ // SB
PADK = 256
KW = PADK + SB
NEG = -1e30
QSCALE = (DH ** -0.5) * math.log2(math.e)


def _head_loc(h):
    lo = DH * h
    t = lo // 128
    if (lo + DH - 1) // 128 == t:
        return t, lo - 128 * t
    lo2 = lo - 64
    t2 = lo2 // 128
    return 5 + t2, lo2 - 128 * t2


def _kernel(x_ref, gw_ref, wqkv_hbm, wo_hbm, w1_hbm, w2_hbm, o_ref,
            wqkv_v, wo_v, w1_v, w2_v, sems, q_s, k_s, vt_s, ot_s):
    step = pl.program_id(0)
    bf16 = jnp.bfloat16
    f32 = jnp.float32

    c_qkv = pltpu.make_async_copy(wqkv_hbm, wqkv_v, sems.at[0])
    c_w1 = pltpu.make_async_copy(w1_hbm, w1_v, sems.at[1])
    c_w2 = pltpu.make_async_copy(w2_hbm, w2_v, sems.at[2])
    c_wo = pltpu.make_async_copy(wo_hbm, wo_v, sems.at[3])

    @pl.when(step == 0)
    def _():
        c_qkv.start()
        c_w1.start()
        c_w2.start()
        c_wo.start()
        k_s[0:PADK, :] = jnp.zeros((PADK, k_s.shape[1]), bf16)
        vt_s[0:2] = jnp.zeros((2, D, 128), bf16)
        c_qkv.wait()

    x = x_ref[...]
    qkv = jnp.dot(x, wqkv_v[...], preferred_element_type=f32)
    q = qkv[:, 0:D] * QSCALE
    k = qkv[:, D:2 * D]
    v = qkv[:, 2 * D:3 * D]
    q_s[:, 0:D] = q.astype(bf16)
    q_s[:, D:D + 512] = q[:, 64:576].astype(bf16)
    row0 = pl.multiple_of(PADK + step * TQ, 128)
    k_s[pl.ds(row0, TQ), 0:D] = k.astype(bf16)
    k_s[pl.ds(row0, TQ), D:D + 512] = k[:, 64:576].astype(bf16)
    vt = v.T
    for j in range(NSB):
        vt_s[2 + step * NSB + j] = vt[:, 128 * j:128 * (j + 1)].astype(bf16)

    def sub(i, carry):
        blk = step * NSB + i
        r = lax.broadcasted_iota(jnp.int32, (KW, SB), 0)
        c = lax.broadcasted_iota(jnp.int32, (KW, SB), 1)
        dqk = PADK + c - r
        valid = (dqk >= 0) & (dqk < W) & (r >= PADK - blk * SB)
        bias = jnp.where(valid, 0.0, NEG).astype(f32)
        krow = pl.multiple_of(blk * SB, 128)
        qrow = pl.multiple_of(i * SB, 128)
        lane = lax.broadcasted_iota(jnp.int32, (SB, 128), 1)
        row8 = lax.broadcasted_iota(jnp.int32, (8, SB), 0)
        for g in range(H // 4):
            os_ = []
            for hh in range(4):
                h = 4 * g + hh
                t, off = _head_loc(h)
                kt = k_s[pl.ds(krow, KW), 128 * t:128 * (t + 1)]
                qt = q_s[pl.ds(qrow, SB), 128 * t:128 * (t + 1)]
                qm = jnp.where((lane >= off) & (lane < off + DH), qt, jnp.zeros_like(qt))
                s = lax.dot_general(kt, qm, (((1,), (1,)), ((), ())),
                                    preferred_element_type=f32) + bias
                m = jnp.max(s, axis=0, keepdims=True)
                p = jnp.exp2(s - m)
                l = jnp.sum(p, axis=0, keepdims=True)
                r0 = 16 * ((DH * h) // 16)
                vth = jnp.concatenate(
                    [vt_s[blk + tt, r0:r0 + 32, :] for tt in range(3)], axis=1)
                o = jnp.dot(vth, p.astype(bf16), preferred_element_type=f32)
                os_.append(o * (1.0 / l))
            o0, o1, o2, o3 = os_
            og = jnp.concatenate([
                o0[0:16],
                jnp.where(row8 < 4, o0[16:24], o1[0:8]),
                o1[8:24],
                o2[8:24],
                jnp.where(row8 < 4, o2[24:32], o3[8:16]),
                o3[16:32]], axis=0)
            ot_s[i, 80 * g:80 * (g + 1), :] = og.astype(bf16)
        return carry

    lax.fori_loop(0, NSB, sub, 0)

    @pl.when(step == 0)
    def _():
        c_w1.wait()
        c_w2.wait()
        c_wo.wait()

    hdn = jnp.dot(x, w1_v[...], preferred_element_type=f32)
    hdn = hdn * jax.nn.sigmoid(hdn)
    b = jnp.dot(hdn.astype(bf16), w2_v[...], preferred_element_type=f32)

    ot = jnp.concatenate([ot_s[j] for j in range(NSB)], axis=1)
    a = lax.dot_general(ot, wo_v[...], (((0,), (0,)), ((), ())),
                        preferred_element_type=f32)

    gl = jnp.sum(x.astype(f32) * gw_ref[...].astype(f32), axis=-1, keepdims=True)
    g = jax.nn.sigmoid(gl)
    o_ref[...] = (g * a + (1.0 - g) * b).astype(o_ref.dtype)


@jax.jit
def pallas_gated_mix__sliding_block__dense_activation_silu__prompt_kernel(
    A_x: jax.Array,
    A_wqkv: jax.Array,
    A_wo: jax.Array,
    B_x: jax.Array,
    B_w1: jax.Array,
    B_w2: jax.Array,
    gate_w: jax.Array,
):
    x = A_x.reshape(S, D)
    gw = gate_w.reshape(1, D)
    bf16 = jnp.bfloat16
    out = pl.pallas_call(
        _kernel,
        grid=(S // TQ,),
        in_specs=[
            pl.BlockSpec((TQ, D), lambda i: (i, 0)),
            pl.BlockSpec((1, D), lambda i: (0, 0)),
            pl.BlockSpec(memory_space=pl.ANY),
            pl.BlockSpec(memory_space=pl.ANY),
            pl.BlockSpec(memory_space=pl.ANY),
            pl.BlockSpec(memory_space=pl.ANY),
        ],
        out_specs=pl.BlockSpec((TQ, D), lambda i: (i, 0)),
        out_shape=jax.ShapeDtypeStruct((S, D), bf16),
        scratch_shapes=[
            pltpu.VMEM((D, 3 * D), bf16),
            pltpu.VMEM((D, D), bf16),
            pltpu.VMEM((D, F), bf16),
            pltpu.VMEM((F, D), bf16),
            pltpu.SemaphoreType.DMA((4,)),
            pltpu.VMEM((TQ, D + 512), bf16),
            pltpu.VMEM((PADK + S, D + 512), bf16),
            pltpu.VMEM((2 + S // 128, D, 128), bf16),
            pltpu.VMEM((NSB, D, 128), bf16),
        ],
        compiler_params=pltpu.CompilerParams(
            dimension_semantics=("arbitrary",),
            vmem_limit_bytes=96 * 1024 * 1024,
        ),
    )(x, gw, A_wqkv, A_wo, B_w1, B_w2)
    return out.reshape(1, S, D)
```

```python
import math

import jax
import jax.numpy as jnp
from jax import lax
import jax.experimental.pallas as pl
import jax.experimental.pallas.tpu as pltpu

S, D, F, H, DH, W = 2048, 640, 1536, 32, 20, 256
TQ = 512
NSTEP = S // TQ
SB = 128
NSB = TQ // SB
PADK = 256
KW = PADK + SB
NEG = -1e30
QSCALE = (DH ** -0.5) * math.log2(math.e)
NG = H // 4
QKV_SPLIT = 512


def _kernel(x_hbm, gw_hbm, wqkv_hbm, wo_hbm, w1_hbm, w2_hbm, o_ref,
            x_v, gw_v, wqkv_v, wo_v, w1_v, w2_v, sems, q_s, k_s, vt_s, ot_s, s_buf, m_s):
    step = pl.program_id(0)
    bf16 = jnp.bfloat16
    f32 = jnp.float32

    c_qkv = [pltpu.make_async_copy(wqkv_hbm.at[:, lo:hi], wqkv_v.at[:, lo:hi], sems.at[j])
             for j, (lo, hi) in enumerate(((0, QKV_SPLIT), (QKV_SPLIT, 3 * D)))]
    c_w1 = pltpu.make_async_copy(w1_hbm, w1_v, sems.at[2])
    c_w2 = pltpu.make_async_copy(w2_hbm, w2_v, sems.at[3])
    c_wo = pltpu.make_async_copy(wo_hbm, wo_v, sems.at[4])
    c_gw = pltpu.make_async_copy(gw_hbm, gw_v, sems.at[5])
    c_x = [pltpu.make_async_copy(x_hbm.at[TQ * j:TQ * (j + 1)], x_v.at[j], sems.at[6 + j])
           for j in range(NSTEP)]

    def put_qkv(qkv, st):
        row0 = pl.multiple_of(PADK + st * TQ, 128)
        flag = lax.broadcasted_iota(jnp.int32, (TQ, 128), 1) == 127
        for g in range(NG):
            q_s[:, 128 * g:128 * (g + 1)] = jnp.where(
                flag, 1.0, qkv[:, 80 * g:80 * g + 128] * QSCALE).astype(bf16)
            k_s[pl.ds(row0, TQ), 128 * g:128 * (g + 1)] = jnp.where(
                flag, 0.0, qkv[:, D + 80 * g:D + 80 * g + 128]).astype(bf16)
        vt = qkv[:, 2 * D:3 * D].T
        for j in range(NSB):
            vt_s[2 + st * NSB + j] = vt[:, 128 * j:128 * (j + 1)].astype(bf16)

    def qk(g, i, st):
        r = lax.broadcasted_iota(jnp.int32, (SB, 4 * SB), 0)
        c = lax.broadcasted_iota(jnp.int32, (SB, 4 * SB), 1) % SB
        tri = r > c
        lane = lax.broadcasted_iota(jnp.int32, (4 * SB, 128), 1)
        rowh = lax.broadcasted_iota(jnp.int32, (4 * SB, 128), 0) // SB
        hmask = ((lane >= rowh * DH) & (lane < rowh * DH + DH)) | (lane == 127)
        krow = pl.multiple_of((st * NSB + i) * SB, 128)
        qrow = pl.multiple_of(i * SB, 128)
        kt = k_s[pl.ds(krow, KW), 128 * g:128 * (g + 1)]
        qt = q_s[pl.ds(qrow, SB), 128 * g:128 * (g + 1)]
        qt4 = jnp.concatenate([qt] * 4, axis=0)
        qm = jnp.where(hmask, qt4, jnp.zeros_like(qt4))
        s = lax.dot_general(kt, qm, (((1,), (1,)), ((), ())),
                            preferred_element_type=f32)
        sm = jnp.concatenate([jnp.where(tri, s[0:SB], s[2 * SB:3 * SB]), s[SB:2 * SB]], axis=0)
        s_buf[g % 2] = sm
        return jnp.max(sm, axis=0, keepdims=True)

    @pl.when(step == 0)
    def _():
        c_x[0].start()
        for c in c_qkv:
            c.start()
        c_x[1].start()
        c_w1.start()
        c_w2.start()
        c_wo.start()
        c_gw.start()
        for c in c_x[2:]:
            c.start()
        lz = lax.broadcasted_iota(jnp.int32, (PADK, k_s.shape[1]), 1) % 128
        k_s[0:PADK, :] = jnp.where(lz == 127, NEG, 0.0).astype(bf16)
        vt_s[0:2] = jnp.zeros((2, D, 128), bf16)
        c_x[0].wait()
        xx = x_v[0]
        c_qkv[0].wait()
        r1 = jnp.dot(xx, wqkv_v[:, 0:QKV_SPLIT], preferred_element_type=f32)
        c_qkv[1].wait()
        r2 = jnp.dot(xx, wqkv_v[:, QKV_SPLIT:3 * D], preferred_element_type=f32)
        put_qkv(jnp.concatenate([r1, r2], axis=1), 0)
        m_s[...] = qk(0, 0, 0)

    def sub(i, m_next):
        blk = step * NSB + i
        tri1 = (lax.broadcasted_iota(jnp.int32, (SB, SB), 0)
                > lax.broadcasted_iota(jnp.int32, (SB, SB), 1))
        row8 = lax.broadcasted_iota(jnp.int32, (8, SB), 0)
        for g in range(NG):
            m = m_next
            if g + 1 < NG:
                m_next = qk(g + 1, i, step)
            else:
                m_next = qk(0, jnp.minimum(i + 1, NSB - 1), step)
            os_ = []
            for hh in range(4):
                h = 4 * g + hh
                cs = slice(128 * hh, 128 * (hh + 1))
                p = jnp.exp2(s_buf[g % 2, :, cs] - m[:, cs])
                linv = 1.0 / jnp.sum(p, axis=0, keepdims=True)
                pm = p[0:SB]
                pfull = jnp.concatenate([jnp.where(tri1, pm, 0.0), p[SB:2 * SB],
                                         jnp.where(tri1, 0.0, pm)], axis=0).astype(bf16)
                r0 = 16 * ((DH * h) // 16)
                vth = jnp.concatenate(
                    [vt_s[blk + tt, r0:r0 + 32, :] for tt in range(3)], axis=1)
                o = jnp.dot(vth, pfull, preferred_element_type=f32)
                os_.append(o * linv)
            m_next = m_next + 0.0 * jnp.concatenate([o[24:25, :] for o in os_], axis=1)
            o0, o1, o2, o3 = os_
            og = jnp.concatenate([
                o0[0:16],
                jnp.where(row8 < 4, o0[16:24], o1[0:8]),
                o1[8:24],
                o2[8:24],
                jnp.where(row8 < 4, o2[24:32], o3[8:16]),
                o3[16:32]], axis=0)
            ot_s[i, 80 * g:80 * (g + 1), :] = og.astype(bf16)
        return m_next

    lax.fori_loop(0, NSB, sub, m_s[...], unroll=2)

    @pl.when(step == 0)
    def _():
        c_w1.wait()
        c_w2.wait()
        c_wo.wait()
        c_gw.wait()
        for c in c_x[1:]:
            c.wait()

    def dense(with_next):
        x = x_v[step]
        if with_next:
            put_qkv(jnp.dot(x_v[step + 1], wqkv_v[...], preferred_element_type=f32), step + 1)
        hdn = jnp.dot(x, w1_v[...], preferred_element_type=f32)
        hdn = hdn * jax.nn.sigmoid(hdn)
        b = jnp.dot(hdn.astype(bf16), w2_v[...], preferred_element_type=f32)

        ot = jnp.concatenate([ot_s[j] for j in range(NSB)], axis=1)
        a = lax.dot_general(ot, wo_v[...], (((0,), (0,)), ((), ())),
                            preferred_element_type=f32)

        gl = jnp.sum(x.astype(f32) * gw_v[...].astype(f32)[None, :], axis=-1, keepdims=True)
        g = jax.nn.sigmoid(gl)
        o_ref[...] = (g * a + (1.0 - g) * b).astype(o_ref.dtype)
        if with_next:
            m_s[...] = qk(0, 0, step + 1)

    @pl.when(step < NSTEP - 1)
    def _():
        dense(True)

    @pl.when(step == NSTEP - 1)
    def _():
        dense(False)


@jax.jit
def pallas_gated_mix__sliding_block__dense_activation_silu__prompt_kernel(
    A_x: jax.Array,
    A_wqkv: jax.Array,
    A_wo: jax.Array,
    B_x: jax.Array,
    B_w1: jax.Array,
    B_w2: jax.Array,
    gate_w: jax.Array,
):
    x = A_x.reshape(S, D)
    bf16 = jnp.bfloat16
    out = pl.pallas_call(
        _kernel,
        grid=(NSTEP,),
        in_specs=[pl.BlockSpec(memory_space=pl.ANY)] * 6,
        out_specs=pl.BlockSpec((TQ, D), lambda i: (i, 0)),
        out_shape=jax.ShapeDtypeStruct((S, D), bf16),
        scratch_shapes=[
            pltpu.VMEM((NSTEP, TQ, D), bf16),
            pltpu.VMEM((D,), bf16),
            pltpu.VMEM((D, 3 * D), bf16),
            pltpu.VMEM((D, D), bf16),
            pltpu.VMEM((D, F), bf16),
            pltpu.VMEM((F, D), bf16),
            pltpu.SemaphoreType.DMA((6 + NSTEP,)),
            pltpu.VMEM((TQ, 128 * NG), bf16),
            pltpu.VMEM((PADK + S, 128 * NG), bf16),
            pltpu.VMEM((2 + S // 128, D, 128), bf16),
            pltpu.VMEM((NSB, D, 128), bf16),
            pltpu.VMEM((2, 2 * SB, 4 * SB), jnp.float32),
            pltpu.VMEM((1, 4 * SB), jnp.float32),
        ],
        compiler_params=pltpu.CompilerParams(
            dimension_semantics=("arbitrary",),
            vmem_limit_bytes=96 * 1024 * 1024,
        ),
    )(x, gate_w, A_wqkv, A_wo, B_w1, B_w2)
    return out.reshape(1, S, D)
```
